```python
import jax
import jax.numpy as jnp

def _softmax(x, axis=-1):
    return jax.nn.softmax(x, axis=axis)
def _gelu(x):
    return jax.nn.gelu(x, approximate=True)
def _silu(x):
    return jax.nn.silu(x)
def _sigmoid(x):
    return jax.nn.sigmoid(x)
def _layernorm(x, axis=-1, eps=1e-5):
    m = jnp.mean(x, axis=axis, keepdims=True)
    v = jnp.var(x, axis=axis, keepdims=True)
    return (x - m) / jnp.sqrt(v + eps)
def _scatter_add(tgt, idx, src, axis=0):
    return tgt.at[idx].add(src)
def _segment_sum(src, seg, n):
    return jax.ops.segment_sum(src, seg, n)
class _Rng:
    def __init__(self, key):
        self._k = key
    def _next(self):
        self._k, sub = jax.random.split(self._k)
        return sub
    def normal(self, shape):
        return jax.random.normal(self._next(), shape, dtype=jnp.bfloat16)
    def randint(self, lo, hi, shape):
        return jax.random.randint(self._next(), shape, lo, hi, dtype=jnp.int32)
    def uniform(self, shape, lo=0.0, hi=1.0):
        return jax.random.uniform(self._next(), shape, jnp.bfloat16, lo, hi)
    def permutation(self, n):
        return jax.random.permutation(self._next(), n)


kernel_name = 'standalone__depthwise_separable__vision'

def setup_inputs():
    _rng = _Rng(jax.random.key(int.from_bytes(__import__("os").urandom(4), "little")))
    _w = (lambda a: (lambda t: t.astype(jnp.bfloat16) if jnp.issubdtype(t.dtype, jnp.floating) else t)(jnp.asarray(a)))
    H = W = 384
    C = 384
    k = 1
    return {
        "x": _w((lambda *s: _rng.normal(s) * 0.05)(1, H, W, C)),
        "dw": _w((lambda *s: _rng.normal(s) * 0.05)(k, k, C)),
        "pw": _w((lambda *s: _rng.normal(s) * 0.05)(C, C)),
    }

def reference(x, dw, pw):
    B, H, W, C = x.shape
    k = dw.shape[0]
    pad = k // 2
    xp = jnp.pad(x, ((0,0),(pad,pad),(pad,pad),(0,0)))
    out = jnp.zeros_like(x)
    for i in range(k):
        for j in range(k):
            out = out + xp[:, i:i+H, j:j+W, :] * dw[i, j][None, None, None, :]
    return jnp.einsum('bhwc,cd->bhwd', out, pw)
```

```python
import jax
import jax.numpy as jnp
from jax import lax
import jax.experimental.pallas as pl
import jax.experimental.pallas.tpu as pltpu

_TM = 64
_S = 36
_B = 16


@jax.jit
def pallas_standalone__depthwise_separable__vision_kernel(
    x: jax.Array,
    dw: jax.Array,
    pw: jax.Array,
):
    bsz, h, w, c = x.shape
    assert dw.shape == (1, 1, c), "kernel is specialised to a 1x1 depthwise filter"
    assert pw.shape == (c, c)
    m = bsz * h * w
    tm, s, b = _TM, _S, _B
    a = m // (s * b * tm)
    assert a * s * b * tm == m
    n = a * b
    rows = s * tm
    j1 = (n * 19) // 32

    def kernel(x_hbm, dw_hbm, pw_hbm, o_hbm, buf, dw_v, pw_v, rsem, wsem, psem):
        def rd(i):
            return pltpu.make_async_copy(
                x_hbm.at[i // b, :, i % b], buf.at[i], rsem.at[i])

        def wr(i):
            return pltpu.make_async_copy(
                buf.at[i], o_hbm.at[i // b, :, i % b], wsem.at[i])

        def each(lo, hi, fn):
            def body(i, carry):
                fn(i)
                return carry
            lax.fori_loop(lo, hi, body, 0)

        cp_dw = pltpu.make_async_copy(dw_hbm, dw_v, psem.at[0])
        cp_pw = pltpu.make_async_copy(pw_hbm, pw_v, psem.at[1])
        cp_dw.start()
        cp_pw.start()
        each(0, n, lambda i: rd(i).start())
        cp_dw.wait()
        cp_pw.wait()

        def step(i):
            @pl.when(i < j1)
            def _():
                rd(i).wait()

            @pl.when(i == j1)
            def _():
                each(j1, n, lambda j: rd(j).wait())
                each(0, j1, lambda j: wr(j).start())

            xs = buf[i].reshape(rows, c) * dw_v[...]
            y = jnp.dot(xs, pw_v[...], preferred_element_type=jnp.float32)
            buf[i] = y.astype(buf.dtype).reshape(s, tm, c)

            @pl.when(i >= j1)
            def _():
                wr(i).start()

        each(0, n, step)
        each(0, n, lambda j: wr(j).wait())

    out = pl.pallas_call(
        kernel,
        in_specs=[pl.BlockSpec(memory_space=pl.ANY)] * 3,
        out_specs=pl.BlockSpec(memory_space=pl.ANY),
        out_shape=jax.ShapeDtypeStruct((a, s, b, tm, c), x.dtype),
        scratch_shapes=[
            pltpu.VMEM((n, s, tm, c), x.dtype),
            pltpu.VMEM((1, c), dw.dtype),
            pltpu.VMEM((c, c), pw.dtype),
            pltpu.SemaphoreType.DMA((n,)),
            pltpu.SemaphoreType.DMA((n,)),
            pltpu.SemaphoreType.DMA((2,)),
        ],
        compiler_params=pltpu.CompilerParams(vmem_limit_bytes=124 * 1024 * 1024),
    )(x.reshape(a, s, b, tm, c), dw.reshape(1, c), pw)
    return out.reshape(x.shape)
```

```python
import jax
import jax.numpy as jnp
from jax import lax
import jax.experimental.pallas as pl
import jax.experimental.pallas.tpu as pltpu

_TM = 32
_S = 6
_NJ = 8
_NB = 16
_LEAD = 48
_RATE = 16


@jax.jit
def pallas_standalone__depthwise_separable__vision_kernel(
    x: jax.Array,
    dw: jax.Array,
    pw: jax.Array,
):
    bsz, h, w, c = x.shape
    assert dw.shape == (1, 1, c), "kernel is specialised to a 1x1 depthwise filter"
    assert pw.shape == (c, c)
    m = bsz * h * w
    tm, s, nj, nb, lead, rate = _TM, _S, _NJ, _NB, _LEAD, _RATE
    na = m // (s * nb * nj * tm)
    assert na * s * nb * nj * tm == m
    view = (na, s, nb, nj, tm, c)
    n = na * nb
    nw = n * nj
    rows = s * nj * tm
    j1 = (n * 9) // 16
    groups = [0, nb // 2] + [nb * a for a in range(1, na + 1)]
    ng = len(groups) - 1
    assert lead <= nj * j1
    assert all(lead + rate * (i - j1 + 1) <= nj * (i + 1) for i in range(j1, n))

    def kernel(x_hbm, dw_hbm, pw_hbm, o_hbm, buf, dw_v, pw_v, rsem, wsem):
        def rd(g):
            lo, hi = groups[g], groups[g + 1]
            if lo % nb == 0 and hi % nb == 0:
                sl = (slice(lo // nb, hi // nb),)
            else:
                sl = (lo // nb, slice(None), slice(lo % nb, (hi - 1) % nb + 1))
            return pltpu.make_async_copy(x_hbm.at[sl], buf.at[sl], rsem.at[g])

        def wr(k):
            a, bb, j = k // (nb * nj), (k // nj) % nb, k % nj
            return pltpu.make_async_copy(
                buf.at[a, :, bb, j], o_hbm.at[a, :, bb, j], wsem.at[0])

        def each(lo, hi, fn):
            def body(i, carry):
                fn(i)
                return carry
            lax.fori_loop(lo, hi, body, 0)

        def wr_next(k):
            wr(k - lead).wait()
            wr(k).start()

        cp_dw = pltpu.make_async_copy(dw_hbm, dw_v, rsem.at[ng])
        cp_pw = pltpu.make_async_copy(pw_hbm, pw_v, rsem.at[ng])
        cp_dw.start()
        cp_pw.start()
        for g in range(ng):
            rd(g).start()
        cp_dw.wait()
        cp_pw.wait()

        def step(i):
            for g in range(ng):
                if groups[g] < j1:
                    pl.when(i == groups[g])(rd(g).wait)

            @pl.when(i == j1)
            def _():
                for g in range(ng):
                    if groups[g] >= j1:
                        rd(g).wait()
                each(0, lead, lambda k: wr(k).start())

            a, bb = i // nb, i % nb
            xs = buf[a, :, bb].reshape(rows, c) * dw_v[...]
            y = jnp.dot(xs, pw_v[...], preferred_element_type=jnp.float32)
            buf[a, :, bb] = y.astype(buf.dtype).reshape(s, nj, tm, c)

            @pl.when(i >= j1)
            def _():
                k0 = lead + rate * (i - j1)
                each(k0, k0 + rate, wr_next)

        each(0, n, step)
        each(lead + rate * (n - j1), nw, wr_next)
        each(nw - lead, nw, lambda k: wr(k).wait())

    out = pl.pallas_call(
        kernel,
        in_specs=[pl.BlockSpec(memory_space=pl.ANY)] * 3,
        out_specs=pl.BlockSpec(memory_space=pl.ANY),
        out_shape=jax.ShapeDtypeStruct(view, x.dtype),
        scratch_shapes=[
            pltpu.VMEM(view, x.dtype),
            pltpu.VMEM((1, c), dw.dtype),
            pltpu.VMEM((c, c), pw.dtype),
            pltpu.SemaphoreType.DMA((ng + 1,)),
            pltpu.SemaphoreType.DMA((1,)),
        ],
        compiler_params=pltpu.CompilerParams(vmem_limit_bytes=124 * 1024 * 1024),
    )(x.reshape(view), dw.reshape(1, c), pw)
    return out.reshape(x.shape)
```

```python
import jax
import jax.numpy as jnp
from jax import lax
import jax.experimental.pallas as pl
import jax.experimental.pallas.tpu as pltpu

_S = 6
_R = 2048
_T = 16
_PIECE = 128
_KP = 15
_NS = 3
_TAIL = 6
_LEAD = 64
_KW = 31


def _log2(v):
    assert v & (v - 1) == 0
    return v.bit_length() - 1


@jax.jit
def pallas_standalone__depthwise_separable__vision_kernel(
    x: jax.Array,
    dw: jax.Array,
    pw: jax.Array,
):
    bsz, h, w, c = x.shape
    assert dw.shape == (1, 1, c), "kernel is specialised to a 1x1 depthwise filter"
    assert pw.shape == (c, c)
    m = bsz * h * w
    s, r, t, pr = _S, _R, _T, _PIECE
    kp, ns, tail, lead, kw = _KP, _NS, _TAIL, _LEAD, _KW
    na = m // (s * r)
    assert na * s * r == m and na % 2 == 0
    view = (na, s, r, c)
    per_a = r // t
    ppa = r // pr
    n = na * ppa // 2
    nw = na * per_a
    npair = nw // 2
    ppc = pr // t
    nb = 1 + (npair - tail - ppc) // kp
    k0 = npair - tail - (nb - 1) * kp
    j1 = nb - 2
    jsw = -(-j1 // ppa) * ppa
    tail_sem, wr_sem = ns, ns + 1

    assert all(k0 + i * kp >= (i + 1) * ppc for i in range(j1))
    assert nb - ns < j1

    def writable(done):
        if done <= jsw:
            return 2 * (done // ppa) * per_a + (done % ppa) * ppc
        return 2 * done * ppc

    assert lead <= writable(j1)
    assert all(lead + kw * (i - j1 + 1) <= writable(i + 1) for i in range(j1, n))

    def kernel(x_hbm, dw_hbm, pw_hbm, o_hbm, buf, dw_v, pw_v, sem):
        def rows(blk, size):
            start = blk * size
            if not isinstance(start, int):
                start = pl.multiple_of(start, size)
            return pl.ds(start, size)

        def rd_start(p, slot):
            g, blk = p >> _log2(per_a), p & (per_a - 1)
            for prio in (1, 0):
                sl = (2 * g + prio, slice(None), rows(blk, t))
                pltpu.make_async_copy(
                    x_hbm.at[sl], buf.at[sl], sem.at[slot]).start(priority=prio)

        def rd_wait(pairs, slot):
            sl = (slice(0, 2), slice(None), pl.ds(0, pairs * t))
            pltpu.make_async_copy(x_hbm.at[sl], buf.at[sl], sem.at[slot]).wait()

        def wr_start(k):
            sl = (k >> _log2(per_a), slice(None), rows(k & (per_a - 1), t))
            pltpu.make_async_copy(buf.at[sl], o_hbm.at[sl], sem.at[wr_sem]).start()

        def wr_wait(count):
            sl = (0, slice(None), pl.ds(0, count * t))
            pltpu.make_async_copy(buf.at[sl], o_hbm.at[sl], sem.at[wr_sem]).wait()

        def each(lo, hi, fn, unroll=1):
            def body(i, carry):
                fn(i)
                return carry
            lax.fori_loop(lo, hi, body, 0, unroll=unroll)

        cp_dw = pltpu.make_async_copy(dw_hbm, dw_v, sem.at[0])
        cp_pw = pltpu.make_async_copy(pw_hbm, pw_v, sem.at[0])
        cp_dw.start()
        cp_pw.start()
        each(0, k0, lambda p: rd_start(p, 0))
        for b in range(1, ns):
            each(k0 + (b - 1) * kp, k0 + b * kp, lambda p, b=b: rd_start(p, b))
        cp_dw.wait()
        cp_pw.wait()
        rd_wait(k0, 0)

        def step(i, slot):
            @pl.when(i < j1)
            def _():
                pl.when(i > 0)(lambda: rd_wait(kp, slot))

                @pl.when(i + ns < nb)
                def _():
                    p0 = k0 + (i + ns - 1) * kp
                    for u in range(kp):
                        rd_start(p0 + u, slot)

                @pl.when(i + ns == nb)
                def _():
                    for u in range(tail):
                        rd_start(npair - tail + u, tail_sem)

            @pl.when(i == j1)
            def _():
                for b in range(j1, nb):
                    rd_wait(kp, b % ns)
                each(0, lead, wr_start, unroll=4)
                rd_wait(tail, tail_sem)

            read_order = i < jsw
            sls = []
            for u in range(2):
                a = jnp.where(read_order, 2 * (i >> _log2(ppa)) + u,
                              i >> (_log2(ppa) - 1))
                blk = jnp.where(read_order, i, 2 * i + u) & (ppa - 1)
                sls.append((a, slice(None), rows(blk, pr)))
            xs = jnp.concatenate([buf[sl].reshape(s * pr, c) for sl in sls], axis=0)
            y = jnp.dot(xs * dw_v[...], pw_v[...], preferred_element_type=jnp.float32)
            y = y.astype(buf.dtype)
            for u, sl in enumerate(sls):
                buf[sl] = y[u * s * pr:(u + 1) * s * pr].reshape(s, pr, c)

            @pl.when(i >= j1)
            def _():
                k_first = lead + kw * (i - j1)
                wr_wait(kw)
                for u in range(kw):
                    wr_start(k_first + u)

            return jnp.where(slot == ns - 1, 0, slot + 1)

        lax.fori_loop(0, n, step, 0)

        def wr_next(k):
            wr_wait(1)
            wr_start(k)

        each(lead + kw * (n - j1), nw, wr_next)
        wr_wait(lead)

    out = pl.pallas_call(
        kernel,
        in_specs=[pl.BlockSpec(memory_space=pl.ANY)] * 3,
        out_specs=pl.BlockSpec(memory_space=pl.ANY),
        out_shape=jax.ShapeDtypeStruct(view, x.dtype),
        scratch_shapes=[
            pltpu.VMEM(view, x.dtype),
            pltpu.VMEM((1, c), dw.dtype),
            pltpu.VMEM((c, c), pw.dtype),
            pltpu.SemaphoreType.DMA((ns + 2,)),
        ],
        compiler_params=pltpu.CompilerParams(
            vmem_limit_bytes=124 * 1024 * 1024,
            disable_bounds_checks=True,
        ),
    )(x.reshape(view), dw.reshape(1, c), pw)
    return out.reshape(x.shape)
```

```python
import jax
import jax.numpy as jnp
from jax import lax
import jax.experimental.pallas as pl
import jax.experimental.pallas.tpu as pltpu

_S = 6
_R = 2048
_TR = 8
_TW = 16
_PIECE = 128
_KP = 30
_NS = 2
_TAIL = 12
_LEAD = 64
_KW = 31


def _log2(v):
    assert v & (v - 1) == 0
    return v.bit_length() - 1


@jax.jit
def pallas_standalone__depthwise_separable__vision_kernel(
    x: jax.Array,
    dw: jax.Array,
    pw: jax.Array,
):
    bsz, h, w, c = x.shape
    assert dw.shape == (1, 1, c), "kernel is specialised to a 1x1 depthwise filter"
    assert pw.shape == (c, c)
    m = bsz * h * w
    s, r, tr, tw, pr = _S, _R, _TR, _TW, _PIECE
    kp, ns, tail, lead, kw = _KP, _NS, _TAIL, _LEAD, _KW
    na = m // (s * r)
    assert na * s * r == m and na % 2 == 0
    view = (na, s, r, c)
    rpa, wpa = r // tr, r // tw
    ppa = r // pr
    n = na * ppa // 2
    nw = na * wpa
    npair = na * rpa // 2
    ppc = pr // tr
    nb = 1 + (npair - tail - ppc) // kp
    k0 = npair - tail - (nb - 1) * kp
    j1 = nb - 2
    jsw = -(-j1 // ppa) * ppa
    tail_sem, wr_sem = ns, ns + 1

    assert all(k0 + i * kp >= (i + 1) * ppc for i in range(j1))
    assert nb - ns <= j1

    def writable(done):
        if done <= jsw:
            return 2 * (done // ppa) * wpa + (done % ppa) * (pr // tw)
        return 2 * done * (pr // tw)

    assert lead <= writable(j1)
    assert all(lead + kw * (i - j1 + 1) <= writable(i + 1) for i in range(j1, n))

    def kernel(x_hbm, dw_hbm, pw_hbm, o_hbm, buf, dw_v, pw_v, sem):
        def rows(blk, size):
            start = blk * size
            if not isinstance(start, int):
                start = pl.multiple_of(start, size)
            return pl.ds(start, size)

        def rd_start(p, slot):
            g, blk = p >> _log2(rpa), p & (rpa - 1)
            for prio in (1, 0):
                sl = (2 * g + prio, slice(None), rows(blk, tr))
                pltpu.make_async_copy(
                    x_hbm.at[sl], buf.at[sl], sem.at[slot]).start(priority=prio)

        def rd_wait(pairs, slot):
            sl = (slice(0, 2), slice(None), pl.ds(0, pairs * tr))
            pltpu.make_async_copy(x_hbm.at[sl], buf.at[sl], sem.at[slot]).wait()

        def wr_start(k):
            sl = (k >> _log2(wpa), slice(None), rows(k & (wpa - 1), tw))
            pltpu.make_async_copy(buf.at[sl], o_hbm.at[sl], sem.at[wr_sem]).start()

        def wr_wait(count):
            sl = (0, slice(None), pl.ds(0, count * tw))
            pltpu.make_async_copy(buf.at[sl], o_hbm.at[sl], sem.at[wr_sem]).wait()

        def each(lo, hi, fn, unroll=1):
            def body(i, carry):
                fn(i)
                return carry
            lax.fori_loop(lo, hi, body, 0, unroll=unroll)

        cp_dw = pltpu.make_async_copy(dw_hbm, dw_v, sem.at[0])
        cp_pw = pltpu.make_async_copy(pw_hbm, pw_v, sem.at[0])
        cp_dw.start()
        cp_pw.start()
        each(0, k0, lambda p: rd_start(p, 0))
        for b in range(1, ns):
            each(k0 + (b - 1) * kp, k0 + b * kp, lambda p, b=b: rd_start(p, b))
        cp_dw.wait()
        cp_pw.wait()
        rd_wait(k0, 0)

        def step(i, slot):
            @pl.when(i < j1)
            def _():
                pl.when(i > 0)(lambda: rd_wait(kp, slot))

                @pl.when(i + ns < nb)
                def _():
                    p0 = k0 + (i + ns - 1) * kp
                    for u in range(kp):
                        rd_start(p0 + u, slot)

            @pl.when(i + ns == nb)
            def _():
                each(npair - tail, npair, lambda p: rd_start(p, tail_sem))

            @pl.when(i == j1)
            def _():
                for b in range(j1, nb):
                    rd_wait(kp, b % ns)
                each(0, lead, wr_start, unroll=4)
                rd_wait(tail, tail_sem)

            read_order = i < jsw
            sls = []
            for u in range(2):
                a = jnp.where(read_order, 2 * (i >> _log2(ppa)) + u,
                              i >> (_log2(ppa) - 1))
                blk = jnp.where(read_order, i, 2 * i + u) & (ppa - 1)
                sls.append((a, slice(None), rows(blk, pr)))
            xs = jnp.concatenate([buf[sl].reshape(s * pr, c) for sl in sls], axis=0)
            y = jnp.dot(xs * dw_v[...], pw_v[...], preferred_element_type=jnp.float32)
            y = y.astype(buf.dtype)
            for u, sl in enumerate(sls):
                buf[sl] = y[u * s * pr:(u + 1) * s * pr].reshape(s, pr, c)

            @pl.when(i >= j1)
            def _():
                k_first = lead + kw * (i - j1)
                wr_wait(kw)
                for u in range(kw):
                    wr_start(k_first + u)

            return jnp.where(slot == ns - 1, 0, slot + 1)

        lax.fori_loop(0, n, step, 0)

        def wr_next(k):
            wr_wait(1)
            wr_start(k)

        each(lead + kw * (n - j1), nw, wr_next)
        wr_wait(lead)

    out = pl.pallas_call(
        kernel,
        in_specs=[pl.BlockSpec(memory_space=pl.ANY)] * 3,
        out_specs=pl.BlockSpec(memory_space=pl.ANY),
        out_shape=jax.ShapeDtypeStruct(view, x.dtype),
        scratch_shapes=[
            pltpu.VMEM(view, x.dtype),
            pltpu.VMEM((1, c), dw.dtype),
            pltpu.VMEM((c, c), pw.dtype),
            pltpu.SemaphoreType.DMA((ns + 2,)),
        ],
        compiler_params=pltpu.CompilerParams(
            vmem_limit_bytes=124 * 1024 * 1024,
            disable_bounds_checks=True,
        ),
    )(x.reshape(view), dw.reshape(1, c), pw)
    return out.reshape(x.shape)
```

```python
import jax
import jax.numpy as jnp
from jax import lax
import jax.experimental.pallas as pl
import jax.experimental.pallas.tpu as pltpu

_S = 6
_R = 2048
_TR = 8
_TW = 16
_PIECE = 128
_KP = 30
_NS = 2
_TAIL = 12
_LEAD = 64
_KW = 31


def _log2(v):
    assert v & (v - 1) == 0
    return v.bit_length() - 1


@jax.jit
def pallas_standalone__depthwise_separable__vision_kernel(
    x: jax.Array,
    dw: jax.Array,
    pw: jax.Array,
):
    bsz, h, w, c = x.shape
    assert dw.shape == (1, 1, c), "kernel is specialised to a 1x1 depthwise filter"
    assert pw.shape == (c, c)
    m = bsz * h * w
    s, r, tr, tw, pr = _S, _R, _TR, _TW, _PIECE
    kp, ns, tail, lead, kw = _KP, _NS, _TAIL, _LEAD, _KW
    na = m // (s * r)
    assert na * s * r == m and na % 2 == 0
    view = (na, s, r, c)
    rpa, wpa = r // tr, r // tw
    ppa = r // pr
    n = na * ppa // 2
    nw = na * wpa
    npair = na * rpa // 2
    ppc = pr // tr
    nb = 1 + (npair - tail - ppc) // kp
    k0 = npair - tail - (nb - 1) * kp
    j1 = nb - 2
    jsw = -(-j1 // ppa) * ppa
    tail_sem, wr_sem = ns, ns + 1

    assert all(k0 + i * kp >= (i + 1) * ppc for i in range(j1))
    assert nb - ns <= j1

    def writable(done):
        if done <= jsw:
            return 2 * (done // ppa) * wpa + (done % ppa) * (pr // tw)
        return 2 * done * (pr // tw)

    assert lead <= writable(j1)
    assert all(lead + kw * (i - j1 + 1) <= writable(i + 1) for i in range(j1, n))

    def kernel(x_hbm, dw_hbm, pw_hbm, o_hbm, buf, dw_v, pw_v, sem):
        def rows(blk, size):
            start = blk * size
            if not isinstance(start, int):
                start = pl.multiple_of(start, size)
            return pl.ds(start, size)

        def rd(p, prio, slot):
            g, blk = p >> _log2(rpa), p & (rpa - 1)
            sl = (2 * g + prio, slice(None), rows(blk, tr))
            return pltpu.make_async_copy(x_hbm.at[sl], buf.at[sl], sem.at[slot])

        def rd_start(p, slot):
            for prio in (1, 0):
                rd(p, prio, slot).start(priority=prio)

        def rd_wait(first, pairs, slot):
            for u in range(pairs):
                for prio in (1, 0):
                    rd(first + u, prio, slot).wait()

        def wr(k):
            sl = (k >> _log2(wpa), slice(None), rows(k & (wpa - 1), tw))
            return pltpu.make_async_copy(buf.at[sl], o_hbm.at[sl], sem.at[wr_sem])

        def wr_wait(first, count):
            for u in range(count):
                wr(first + u).wait()

        def each(lo, hi, fn, unroll=1):
            def body(i, carry):
                fn(i)
                return carry
            lax.fori_loop(lo, hi, body, 0, unroll=unroll)

        cp_dw = pltpu.make_async_copy(dw_hbm, dw_v, sem.at[0])
        cp_pw = pltpu.make_async_copy(pw_hbm, pw_v, sem.at[0])
        cp_dw.start()
        cp_pw.start()
        each(0, k0, lambda p: rd_start(p, 0))
        for b in range(1, ns):
            each(k0 + (b - 1) * kp, k0 + b * kp, lambda p, b=b: rd_start(p, b))
        cp_dw.wait()
        cp_pw.wait()
        rd_wait(0, k0, 0)

        def step(i, slot):
            @pl.when(i < j1)
            def _():
                pl.when(i > 0)(lambda: rd_wait(k0 + (i - 1) * kp, kp, slot))

                @pl.when(i + ns < nb)
                def _():
                    p0 = k0 + (i + ns - 1) * kp
                    for u in range(kp):
                        rd_start(p0 + u, slot)

            @pl.when(i + ns == nb)
            def _():
                each(npair - tail, npair, lambda p: rd_start(p, tail_sem))

            @pl.when(i == j1)
            def _():
                for b in range(j1, nb):
                    rd_wait(k0 + (b - 1) * kp, kp, b % ns)
                each(0, lead, lambda k: wr(k).start(), unroll=4)
                rd_wait(npair - tail, tail, tail_sem)

            read_order = i < jsw
            sls = []
            for u in range(2):
                a = jnp.where(read_order, 2 * (i >> _log2(ppa)) + u,
                              i >> (_log2(ppa) - 1))
                blk = jnp.where(read_order, i, 2 * i + u) & (ppa - 1)
                sls.append((a, slice(None), rows(blk, pr)))
            xs = jnp.concatenate([buf[sl].reshape(s * pr, c) for sl in sls], axis=0)
            y = jnp.dot(xs * dw_v[...], pw_v[...], preferred_element_type=jnp.float32)
            y = y.astype(buf.dtype)
            for u, sl in enumerate(sls):
                buf[sl] = y[u * s * pr:(u + 1) * s * pr].reshape(s, pr, c)

            @pl.when(i >= j1)
            def _():
                k_first = lead + kw * (i - j1)
                wr_wait(k_first - lead, kw)
                for u in range(kw):
                    wr(k_first + u).start()

            return jnp.where(slot == ns - 1, 0, slot + 1)

        lax.fori_loop(0, n, step, 0)

        def wr_next(k):
            wr(k - lead).wait()
            wr(k).start()

        each(lead + kw * (n - j1), nw, wr_next)
        wr_wait(nw - lead, lead)

    out = pl.pallas_call(
        kernel,
        in_specs=[pl.BlockSpec(memory_space=pl.ANY)] * 3,
        out_specs=pl.BlockSpec(memory_space=pl.ANY),
        out_shape=jax.ShapeDtypeStruct(view, x.dtype),
        scratch_shapes=[
            pltpu.VMEM(view, x.dtype),
            pltpu.VMEM((1, c), dw.dtype),
            pltpu.VMEM((c, c), pw.dtype),
            pltpu.SemaphoreType.DMA((ns + 2,)),
        ],
        compiler_params=pltpu.CompilerParams(
            vmem_limit_bytes=124 * 1024 * 1024,
            disable_bounds_checks=True,
        ),
    )(x.reshape(view), dw.reshape(1, c), pw)
    return out.reshape(x.shape)
```

```python
import jax
import jax.numpy as jnp
from jax import lax
import jax.experimental.pallas as pl
import jax.experimental.pallas.tpu as pltpu

_LANES = 128
_SUB = 8
_SR = 4096
_RD_STREAMS = 18
_RD_LOW = 16
_RD_ROWS = 16
_WR_STREAMS = 6
_WR_PARTS = (40, 40, 48)
_PIECE = 128
_PIECES = 12
_BLK = 128
_KP = 30
_NS = 2
_TAIL = 8
_LEAD = 24
_KW = 11


def _log2(v):
    assert v & (v - 1) == 0
    return v.bit_length() - 1


@jax.jit
def pallas_standalone__depthwise_separable__vision_kernel(
    x: jax.Array,
    dw: jax.Array,
    pw: jax.Array,
):
    bsz, h, w, c = x.shape
    assert dw.shape == (1, 1, c), "kernel is specialised to a 1x1 depthwise filter"
    assert pw.shape == (c, c)
    m = bsz * h * w
    nc = c // _LANES
    sr, kp, ns, tail, lead, kw = _SR, _KP, _NS, _TAIL, _LEAD, _KW
    nstr = m * nc // sr
    assert nc * _LANES == c and nstr * sr == m * nc
    assert nstr % _RD_STREAMS == 0 and nstr % _WR_STREAMS == 0
    assert _RD_STREAMS % nc == 0 and _WR_STREAMS % nc == 0
    view = (nstr, sr, _LANES)

    prow = _PIECE * nc
    pps = nc * sr // prow
    spans = _RD_STREAMS // nc
    mpc = _PIECES // spans
    cpg = pps // mpc
    rows = _PIECE * _PIECES
    n = m // rows
    assert mpc * spans == _PIECES and cpg * mpc == pps and n * rows == m
    rpg = sr // _RD_ROWS
    npair = nstr // _RD_STREAMS * rpg
    wrow = sum(_WR_PARTS)
    wpg = sr // wrow
    nw = nstr // _WR_STREAMS * wpg
    assert rpg * _RD_ROWS == sr and wpg * wrow == sr

    hop = -(-sr // prow)

    def order(q):
        if isinstance(q, int):
            return q // nc + hop * (q % nc)
        return lax.div(q, nc) + hop * lax.rem(q, nc)

    assert sorted(order(q) for q in range(pps)) == list(range(pps))

    def pairs_needed(i):
        g, j = divmod(i, cpg)
        front = 0
        for q in range(j * mpc, (j + 1) * mpc):
            lo, hi = order(q) * prow, (order(q) + 1) * prow - 1
            front = max(front, sr if lo // sr != hi // sr else hi % sr + 1)
        return g * rpg + -(-front // _RD_ROWS)

    nb = 1 + (npair - tail - pairs_needed(0)) // kp
    k0 = npair - tail - (nb - 1) * kp
    j1 = nb - 2
    jsw = -(-j1 // cpg) * cpg
    tail_sem, wr_sem = ns, ns + 1
    assert all(k0 + i * kp >= pairs_needed(i) for i in range(j1))
    assert nb - ns <= j1

    def writable(done):
        if done <= jsw:
            done -= done % cpg
        return done * _PIECES // (_WR_STREAMS // nc * pps) * wpg

    assert lead <= writable(j1)
    assert all(lead + kw * (i - j1 + 1) <= writable(i + 1) for i in range(j1, n))

    def kernel(x_hbm, dw_hbm, pw_hbm, o_hbm, buf, dw_v, pw_v, sem):
        def ds(start, size, align):
            if not isinstance(start, int):
                start = pl.multiple_of(start, align)
            return pl.ds(start, size)

        def rd(p, slot):
            s0 = (p >> _log2(rpg)) * _RD_STREAMS
            rr = ds((p & (rpg - 1)) * _RD_ROWS, _RD_ROWS, _RD_ROWS)
            low = (pl.ds(s0, _RD_LOW), rr)
            high = (pl.ds(s0 + _RD_LOW, _RD_STREAMS - _RD_LOW), rr)
            return [
                (pltpu.make_async_copy(x_hbm.at[sl], buf.at[sl], sem.at[slot]), prio)
                for sl, prio in ((low, 1), (high, 0))
            ]

        def rd_start(p, slot):
            for cp, prio in rd(p, slot):
                cp.start(priority=prio)

        def rd_wait(first, count, slot):
            for u in range(count):
                for cp, _ in rd(first + u, slot):
                    cp.wait()

        def wr(k):
            streams = pl.ds((k >> _log2(wpg)) * _WR_STREAMS, _WR_STREAMS)
            r0 = (k & (wpg - 1)) * wrow
            cps = []
            for size in _WR_PARTS:
                sl = (streams, ds(r0, size, _SUB))
                cps.append(
                    pltpu.make_async_copy(buf.at[sl], o_hbm.at[sl], sem.at[wr_sem]))
                r0 = r0 + size
            return cps

        def wr_start(k):
            for cp in wr(k):
                cp.start()

        def wr_wait(first, count):
            for u in range(count):
                for cp in wr(first + u):
                    cp.wait()

        def each(lo, hi, fn):
            def body(i, carry):
                fn(i)
                return carry
            lax.fori_loop(lo, hi, body, 0)

        def compute(i):
            read_order = i < jsw
            g, j = i >> _log2(cpg), i & (cpg - 1)
            bpp, bps = prow // _BLK, sr // _BLK
            blocks = []
            for uq in range(mpc):
                piece = order(j * mpc + uq)
                for us in range(spans):
                    p = jnp.where(read_order, (g * spans + us) * pps + piece,
                                  i * _PIECES + uq * spans + us)
                    for v in range(bpp):
                        blk = p * bpp + v
                        blocks.append(
                            (blk >> _log2(bps), ds((blk & (bps - 1)) * _BLK, _BLK, _BLK)))
            tiles = jnp.concatenate([buf[sl] for sl in blocks], axis=0)
            tiles = tiles.astype(jnp.float32).reshape(rows // _SUB, nc, _SUB, _LANES)
            scale = dw_v[...].astype(jnp.float32)
            xs = jnp.concatenate(
                [(tiles[:, b].reshape(rows, _LANES)
                  * scale[:, b * _LANES:(b + 1) * _LANES]).astype(buf.dtype)
                 for b in range(nc)], axis=1)
            y = jnp.dot(xs, pw_v[...], preferred_element_type=jnp.float32)
            y = jnp.concatenate(
                [y[:, b * _LANES:(b + 1) * _LANES].reshape(rows // _SUB, 1, _SUB, _LANES)
                 for b in range(nc)], axis=1)
            y = y.reshape(rows * nc, _LANES).astype(buf.dtype)
            for u, sl in enumerate(blocks):
                buf[sl] = y[u * _BLK:(u + 1) * _BLK]

        cp_dw = pltpu.make_async_copy(dw_hbm, dw_v, sem.at[0])
        cp_pw = pltpu.make_async_copy(pw_hbm, pw_v, sem.at[0])
        cp_dw.start()
        cp_pw.start()
        each(0, k0, lambda p: rd_start(p, 0))
        for b in range(1, ns):
            each(k0 + (b - 1) * kp, k0 + b * kp, lambda p, b=b: rd_start(p, b))
        cp_dw.wait()
        cp_pw.wait()
        rd_wait(0, k0, 0)

        def step(i, slot):
            @pl.when(i < j1)
            def _():
                pl.when(i > 0)(lambda: rd_wait(k0 + (i - 1) * kp, kp, slot))

                @pl.when(i + ns < nb)
                def _():
                    first = k0 + (i + ns - 1) * kp
                    for u in range(kp):
                        rd_start(first + u, slot)

            @pl.when(i + ns == nb)
            def _():
                each(npair - tail, npair, lambda p: rd_start(p, tail_sem))

            @pl.when(i == j1)
            def _():
                for b in range(j1, nb):
                    rd_wait(k0 + (b - 1) * kp, kp, b % ns)
                each(0, lead, wr_start)
                rd_wait(npair - tail, tail, tail_sem)

            compute(i)

            @pl.when(i >= j1)
            def _():
                first = lead + kw * (i - j1)
                wr_wait(first - lead, kw)
                for u in range(kw):
                    wr_start(first + u)

            return jnp.where(slot == ns - 1, 0, slot + 1)

        lax.fori_loop(0, n, step, 0)

        def wr_next(k):
            wr_wait(k - lead, 1)
            wr_start(k)

        each(lead + kw * (n - j1), nw, wr_next)
        wr_wait(nw - lead, lead)

    xt = x.reshape(m // _SUB, _SUB, nc, _LANES).transpose(0, 2, 1, 3).reshape(view)
    out = pl.pallas_call(
        kernel,
        in_specs=[pl.BlockSpec(memory_space=pl.ANY)] * 3,
        out_specs=pl.BlockSpec(memory_space=pl.ANY),
        out_shape=jax.ShapeDtypeStruct(view, x.dtype),
        scratch_shapes=[
            pltpu.VMEM(view, x.dtype),
            pltpu.VMEM((1, c), dw.dtype),
            pltpu.VMEM((c, c), pw.dtype),
            pltpu.SemaphoreType.DMA((ns + 2,)),
        ],
        compiler_params=pltpu.CompilerParams(
            vmem_limit_bytes=124 * 1024 * 1024,
            disable_bounds_checks=True,
        ),
    )(xt, dw.reshape(1, c), pw)
    out = out.reshape(m // _SUB, nc, _SUB, _LANES).transpose(0, 2, 1, 3)
    return out.reshape(x.shape)
```

```python
import jax
import jax.numpy as jnp
from jax import lax
import jax.experimental.pallas as pl
import jax.experimental.pallas.tpu as pltpu

_LANES = 128
_SUB = 8
_SR = 4096
_GROUP = 6
_LOW = 5
_RD_ROWS = 16
_WR_SPANS = 2
_WR_PARTS = (40, 40, 48)
_BAND = 8
_BLK = 128
_PIECES = 2
_KP = 30
_TAIL = 8
_LEAD = 24
_KW = 11


def _log2(v):
    assert v & (v - 1) == 0
    return v.bit_length() - 1


@jax.jit
def pallas_standalone__depthwise_separable__vision_kernel(
    x: jax.Array,
    dw: jax.Array,
    pw: jax.Array,
):
    bsz, h, w, c = x.shape
    assert dw.shape == (1, 1, c), "kernel is specialised to a 1x1 depthwise filter"
    assert pw.shape == (c, c)
    m = bsz * h * w
    nc = c // _LANES
    sr, blk, kp, tail, lead, kw = _SR, _BLK, _KP, _TAIL, _LEAD, _KW
    ng = m // (sr * _GROUP)
    assert nc * _LANES == c and ng * sr * _GROUP == m
    view = (ng * _GROUP, nc, sr, _LANES)

    bps = sr // blk
    cpg = bps // _PIECES
    n = ng * cpg
    pix = blk * _PIECES * _GROUP
    rpg = sr // _RD_ROWS
    npair = ng * rpg
    wsets = _GROUP // _WR_SPANS
    nw = ng * wsets * bps
    banded = nw - wsets * bps
    assert sum(_WR_PARTS) == blk

    hop = -(-bps // nc)

    def order(q):
        if isinstance(q, int):
            return q // nc + hop * (q % nc)
        return lax.div(q, nc) + hop * lax.rem(q, nc)

    rank = {order(q): q for q in range(bps)}
    assert sorted(rank) == list(range(bps))

    def pairs_needed(i):
        g, j = divmod(i, cpg)
        front = max((nc * order(j * _PIECES + u) + v) % bps + 1
                    for u in range(_PIECES) for v in range(nc))
        return g * rpg + front * blk // _RD_ROWS

    def unit(k):
        if isinstance(k, int):
            if k < banded:
                return divmod(k, bps)
            t, v = divmod(k - banded, _BAND)
            return (banded // bps + t % wsets,
                    (t // wsets * _BAND + v + nc - 1) % bps)
        t = jnp.maximum(k - banded, 0) >> _log2(_BAND)
        turn = lax.div(t, wsets) * _BAND + (k & (_BAND - 1)) + nc - 1
        return (jnp.where(k < banded, k >> _log2(bps), banded // bps + lax.rem(t, wsets)),
                jnp.where(k < banded, k, turn) & (bps - 1))

    assert len({unit(k) for k in range(nw)}) == nw

    def chunks_needed(k):
        a, b = unit(k)
        q = max(rank[(s * bps + b) // nc] for s in range(nc))
        return a // wsets * cpg + q // _PIECES + 1

    nb = 1 + (npair - tail - pairs_needed(0)) // kp
    k0 = npair - tail - (nb - 1) * kp
    j1 = nb - 2
    wr_sem = (nb - 1) % 2
    assert all(k0 + i * kp >= pairs_needed(i) for i in range(j1))
    assert lead + kw * (n - j1) <= nw
    assert all(chunks_needed(k) <= j1 + max((k - lead) // kw + 1, 0) for k in range(nw))

    def kernel(x_hbm, dw_hbm, pw_hbm, o_hbm, buf, dw_v, pw_v, sem):
        def ds(start, size, align):
            if not isinstance(start, int):
                start = pl.multiple_of(start, align)
            return pl.ds(start, size)

        def rd(p, slot):
            s0 = (p >> _log2(rpg)) * _GROUP
            rows = ds((p & (rpg - 1)) * _RD_ROWS, _RD_ROWS, _RD_ROWS)
            low = (pl.ds(s0, _LOW), slice(None), rows)
            high = (pl.ds(s0 + _LOW, _GROUP - _LOW), slice(None), rows)
            return [
                (pltpu.make_async_copy(x_hbm.at[sl], buf.at[sl], sem.at[slot]), prio)
                for sl, prio in ((low, 1), (high, 0))
            ]

        def rd_start(p, slot):
            for cp, prio in rd(p, slot):
                cp.start(priority=prio)

        def rd_wait(first, count, slot):
            for u in range(count):
                for cp, _ in rd(first + u, slot):
                    cp.wait()

        def wr(k):
            a, b = unit(k)
            r0, cps = b * blk, []
            for size in _WR_PARTS:
                sl = (pl.ds(a * _WR_SPANS, _WR_SPANS), slice(None), ds(r0, size, _SUB))
                cps.append(
                    pltpu.make_async_copy(buf.at[sl], o_hbm.at[sl], sem.at[wr_sem]))
                r0 = r0 + size
            return cps

        def wr_start(k):
            for cp in wr(k):
                cp.start()

        def wr_wait(first, count):
            for u in range(count):
                for cp in wr(first + u):
                    cp.wait()

        def each(lo, hi, fn):
            def body(i, carry):
                fn(i)
                return carry
            lax.fori_loop(lo, hi, body, 0)

        def compute(i):
            spans = pl.ds((i >> _log2(cpg)) * _GROUP, _GROUP)
            blocks = []
            for u in range(_PIECES):
                piece = order((i & (cpg - 1)) * _PIECES + u)
                for v in range(nc):
                    b = nc * piece + v
                    blocks.append(
                        (spans, b >> _log2(bps), ds((b & (bps - 1)) * blk, blk, blk)))
            tiles = jnp.concatenate([buf[sl] for sl in blocks], axis=1)
            tiles = tiles.astype(jnp.float32).reshape(pix // _SUB, nc, _SUB, _LANES)
            scale = dw_v[...].astype(jnp.float32)
            xs = jnp.concatenate(
                [(tiles[:, b].reshape(pix, _LANES)
                  * scale[:, b * _LANES:(b + 1) * _LANES]).astype(buf.dtype)
                 for b in range(nc)], axis=1)
            y = jnp.dot(xs, pw_v[...], preferred_element_type=jnp.float32)
            y = jnp.concatenate(
                [y[:, b * _LANES:(b + 1) * _LANES].reshape(pix // _SUB, 1, _SUB, _LANES)
                 for b in range(nc)], axis=1)
            y = y.reshape(_GROUP, len(blocks) * blk, _LANES).astype(buf.dtype)
            for u, sl in enumerate(blocks):
                buf[sl] = y[:, u * blk:(u + 1) * blk]

        cp_dw = pltpu.make_async_copy(dw_hbm, dw_v, sem.at[0])
        cp_pw = pltpu.make_async_copy(pw_hbm, pw_v, sem.at[0])
        cp_dw.start()
        cp_pw.start()
        each(0, k0, lambda p: rd_start(p, 0))
        each(k0, k0 + kp, lambda p: rd_start(p, 1))
        cp_dw.wait()
        cp_pw.wait()
        rd_wait(0, k0, 0)

        def step(i):
            @pl.when(i < j1)
            def _():
                pl.when(i > 0)(lambda: rd_wait(k0 + (i - 1) * kp, kp, i & 1))
                for u in range(kp):
                    rd_start(k0 + (i + 1) * kp + u, i & 1)

            @pl.when(i == j1)
            def _():
                rd_wait(k0 + (j1 - 1) * kp, kp, j1 % 2)
                each(npair - tail, npair, lambda p: rd_start(p, nb % 2))
                rd_wait(k0 + j1 * kp, kp, wr_sem)
                each(0, lead, wr_start)
                rd_wait(npair - tail, tail, nb % 2)

            compute(i)

            @pl.when(i >= j1)
            def _():
                first = lead + kw * (i - j1)
                wr_wait(first - lead, kw)
                for u in range(kw):
                    wr_start(first + u)

        each(0, n, step)

        def wr_next(k):
            wr_wait(k - lead, 1)
            wr_start(k)

        each(lead + kw * (n - j1), nw, wr_next)
        wr_wait(nw - lead, lead)

    xt = x.reshape(m // _SUB, _SUB, nc, _LANES).transpose(0, 2, 1, 3).reshape(view)
    out = pl.pallas_call(
        kernel,
        in_specs=[pl.BlockSpec(memory_space=pl.ANY)] * 3,
        out_specs=pl.BlockSpec(memory_space=pl.ANY),
        out_shape=jax.ShapeDtypeStruct(view, x.dtype),
        scratch_shapes=[
            pltpu.VMEM(view, x.dtype),
            pltpu.VMEM((1, c), dw.dtype),
            pltpu.VMEM((c, c), pw.dtype),
            pltpu.SemaphoreType.DMA((2,)),
        ],
        compiler_params=pltpu.CompilerParams(
            vmem_limit_bytes=124 * 1024 * 1024,
            disable_bounds_checks=True,
        ),
    )(xt, dw.reshape(1, c), pw)
    out = out.reshape(m // _SUB, nc, _SUB, _LANES).transpose(0, 2, 1, 3)
    return out.reshape(x.shape)
```

```python
import jax
import jax.numpy as jnp
from jax import lax
import jax.experimental.pallas as pl
import jax.experimental.pallas.tpu as pltpu

_LANES = 128
_SUB = 8
_SR = 4096
_GROUP = 6
_RD_ROWS = 16
_SKEW = 26
_WR_SPANS = 2
_WR_PARTS = (40, 40, 48)
_BAND = 8
_BLK = 128
_PIECES = 2
_KP = 29
_TAIL = 12
_LEAD = 24
_KW = 11


def _log2(v):
    assert v & (v - 1) == 0
    return v.bit_length() - 1


@jax.jit
def pallas_standalone__depthwise_separable__vision_kernel(
    x: jax.Array,
    dw: jax.Array,
    pw: jax.Array,
):
    bsz, h, w, c = x.shape
    assert dw.shape == (1, 1, c), "kernel is specialised to a 1x1 depthwise filter"
    assert pw.shape == (c, c)
    m = bsz * h * w
    nc = c // _LANES
    sr, blk, skew, kp, tail, lead, kw = _SR, _BLK, _SKEW, _KP, _TAIL, _LEAD, _KW
    ng = m // (sr * _GROUP)
    assert nc * _LANES == c and ng * sr * _GROUP == m
    view = (ng * _GROUP, nc, sr, _LANES)

    bps = sr // blk
    cpg = bps // _PIECES
    n = ng * cpg
    pix = blk * _PIECES * _GROUP
    rpg = sr // _RD_ROWS
    nrd = ng * rpg
    wsets = _GROUP // _WR_SPANS
    nw = ng * wsets * bps
    banded = nw - wsets * bps
    assert sum(_WR_PARTS) == blk

    hop = pow(nc, -1, bps)

    def order(q):
        return (q * hop) & (bps - 1)

    rank = {order(q): q for q in range(bps)}
    assert sorted(rank) == list(range(bps))

    def reads_needed(i):
        g, j = divmod(i, cpg)
        front = max((nc * order(j * _PIECES + u) + v) % bps + 1
                    for u in range(_PIECES) for v in range(nc))
        return g * rpg + front * blk // _RD_ROWS

    def unit(k):
        if isinstance(k, int):
            if k < banded:
                return divmod(k, bps)
            t, v = divmod(k - banded, _BAND)
            return (banded // bps + t % wsets,
                    (t // wsets * _BAND + v + nc - 1) % bps)
        t = jnp.maximum(k - banded, 0) >> _log2(_BAND)
        turn = lax.div(t, wsets) * _BAND + (k & (_BAND - 1)) + nc - 1
        return (jnp.where(k < banded, k >> _log2(bps), banded // bps + lax.rem(t, wsets)),
                jnp.where(k < banded, k, turn) & (bps - 1))

    assert len({unit(k) for k in range(nw)}) == nw

    def chunks_needed(k):
        a, b = unit(k)
        q = max(rank[(s * bps + b) // nc] for s in range(nc))
        return a // wsets * cpg + q // _PIECES + 1

    npair = nrd - skew
    nb = 1 + (npair - tail - reads_needed(0)) // kp
    k0 = npair - tail - (nb - 1) * kp
    j1 = nb - 3
    tail_sem, wr_sem = nb % 3, (nb - 1) % 3
    assert k0 >= kp
    assert all(k0 + i * kp >= reads_needed(i) for i in range(j1))
    assert lead + kw * (n - j1) <= nw
    assert all(chunks_needed(k) <= j1 + max((k - lead) // kw, 0) for k in range(nw))

    def kernel(x_hbm, dw_hbm, pw_hbm, o_hbm, buf, dw_v, pw_v, sem):
        def ds(start, size, align):
            if not isinstance(start, int):
                start = pl.multiple_of(start, align)
            return pl.ds(start, size)

        def rd(q, prio, slot):
            half = _GROUP // 2
            sl = (pl.ds((q >> _log2(rpg)) * _GROUP + (1 - prio) * half, half),
                  slice(None), ds((q & (rpg - 1)) * _RD_ROWS, _RD_ROWS, _RD_ROWS))
            return pltpu.make_async_copy(x_hbm.at[sl], buf.at[sl], sem.at[slot])

        def rd_start(p, slot):
            rd(p + skew, 1, slot).start(priority=1)
            rd(p, 0, slot).start(priority=0)

        def rd_wait(first, count, slot):
            for u in range(count):
                rd(first + u + skew, 1, slot).wait()
                rd(first + u, 0, slot).wait()

        def wr(k):
            a, b = unit(k)
            r0, cps = b * blk, []
            for size in _WR_PARTS:
                sl = (pl.ds(a * _WR_SPANS, _WR_SPANS), slice(None), ds(r0, size, _SUB))
                cps.append(
                    pltpu.make_async_copy(buf.at[sl], o_hbm.at[sl], sem.at[wr_sem]))
                r0 = r0 + size
            return cps

        def wr_start(k):
            for cp in wr(k):
                cp.start()

        def wr_wait(first, count):
            for u in range(count):
                for cp in wr(first + u):
                    cp.wait()

        def each(lo, hi, fn):
            def body(i, carry):
                fn(i)
                return carry
            lax.fori_loop(lo, hi, body, 0)

        def compute(i, start_copies):
            spans = pl.ds((i >> _log2(cpg)) * _GROUP, _GROUP)
            blocks = []
            for u in range(_PIECES):
                piece = order((i & (cpg - 1)) * _PIECES + u)
                for v in range(nc):
                    b = nc * piece + v
                    blocks.append(
                        (spans, b >> _log2(bps), ds((b & (bps - 1)) * blk, blk, blk)))
            tiles = jnp.concatenate([buf[sl] for sl in blocks], axis=1)
            start_copies()
            tiles = tiles.astype(jnp.float32).reshape(pix // _SUB, nc, _SUB, _LANES)
            scale = dw_v[...].astype(jnp.float32)
            xs = jnp.concatenate(
                [(tiles[:, b].reshape(pix, _LANES)
                  * scale[:, b * _LANES:(b + 1) * _LANES]).astype(buf.dtype)
                 for b in range(nc)], axis=1)
            y = jnp.dot(xs, pw_v[...], preferred_element_type=jnp.float32)
            y = jnp.concatenate(
                [y[:, b * _LANES:(b + 1) * _LANES].reshape(pix // _SUB, 1, _SUB, _LANES)
                 for b in range(nc)], axis=1)
            y = y.reshape(_GROUP, len(blocks) * blk, _LANES).astype(buf.dtype)
            for u, sl in enumerate(blocks):
                buf[sl] = y[:, u * blk:(u + 1) * blk]

        cp_dw = pltpu.make_async_copy(dw_hbm, dw_v, sem.at[0])
        cp_pw = pltpu.make_async_copy(pw_hbm, pw_v, sem.at[0])
        cp_dw.start()
        cp_pw.start()
        each(0, skew, lambda q: rd(q, 1, 0).start(priority=1))
        each(0, k0, lambda p: rd_start(p, 0))
        each(k0, k0 + kp, lambda p: rd_start(p, 1))
        each(k0 + kp, k0 + 2 * kp, lambda p: rd_start(p, 2))
        cp_dw.wait()
        cp_pw.wait()
        for q in range(skew):
            rd(q, 1, 0).wait()
        rd_wait(0, k0 - kp, 0)

        def read_step(i, slot):
            rd_wait(k0 + (i - 1) * kp, kp, slot)

            def start_copies():
                for u in range(kp):
                    rd_start(k0 + (i + 2) * kp + u, slot)

            compute(i, start_copies)
            return jnp.where(slot == 2, 0, slot + 1)

        lax.fori_loop(0, j1, read_step, 0)

        rd_wait(k0 + (j1 - 1) * kp, kp, tail_sem)
        each(npair - tail, npair, lambda p: rd_start(p, tail_sem))
        each(npair, nrd, lambda q: rd(q, 0, tail_sem).start(priority=0))
        for b in range(j1 + 1, nb):
            rd_wait(k0 + (b - 1) * kp, kp, b % 3)
        each(0, lead, wr_start)
        rd_wait(npair - tail, tail, tail_sem)
        for q in range(npair, nrd):
            rd(q, 0, tail_sem).wait()

        def write_step(i):
            first = lead + kw * (i - j1)
            wr_wait(first - lead, kw)

            def start_copies():
                for u in range(kw):
                    wr_start(first + u)

            compute(i, start_copies)

        each(j1, n, write_step)

        def wr_next(k):
            wr_wait(k - lead, 1)
            wr_start(k)

        each(lead + kw * (n - j1), nw, wr_next)
        wr_wait(nw - lead, lead)

    xt = x.reshape(m // _SUB, _SUB, nc, _LANES).transpose(0, 2, 1, 3).reshape(view)
    out = pl.pallas_call(
        kernel,
        in_specs=[pl.BlockSpec(memory_space=pl.ANY)] * 3,
        out_specs=pl.BlockSpec(memory_space=pl.ANY),
        out_shape=jax.ShapeDtypeStruct(view, x.dtype),
        scratch_shapes=[
            pltpu.VMEM(view, x.dtype),
            pltpu.VMEM((1, c), dw.dtype),
            pltpu.VMEM((c, c), pw.dtype),
            pltpu.SemaphoreType.DMA((3,)),
        ],
        compiler_params=pltpu.CompilerParams(
            vmem_limit_bytes=124 * 1024 * 1024,
            disable_bounds_checks=True,
        ),
    )(xt, dw.reshape(1, c), pw)
    out = out.reshape(m // _SUB, nc, _SUB, _LANES).transpose(0, 2, 1, 3)
    return out.reshape(x.shape)
```

```python
import jax
import jax.numpy as jnp
from jax import lax
import jax.experimental.pallas as pl
import jax.experimental.pallas.tpu as pltpu

_LANES = 128
_SUB = 8
_STRIP = 2048
_BLK = 128
_GROUP = 6
_RD_ROWS = 8
_SKEW = 26
_WR_SPANS = 2
_WR_PARTS = (48, 48, 32)
_BAND = 4
_KP = 29
_TAIL = 12
_LEAD = 24
_KW = 11


def _log2(v):
    assert v & (v - 1) == 0
    return v.bit_length() - 1


@jax.jit
def pallas_standalone__depthwise_separable__vision_kernel(
    x: jax.Array,
    dw: jax.Array,
    pw: jax.Array,
):
    bsz, h, w, c = x.shape
    assert dw.shape == (1, 1, c), "kernel is specialised to a 1x1 depthwise filter"
    assert pw.shape == (c, c)
    m = bsz * h * w
    nc = c // _LANES
    blk, skew, kp, tail, lead, kw = _BLK, _SKEW, _KP, _TAIL, _LEAD, _KW
    ng = m // (2 * _STRIP * _GROUP)
    assert nc * _LANES == c and ng * 2 * _STRIP * _GROUP == m
    view = (ng * _GROUP, nc, 2, _STRIP, _LANES)

    bps = _STRIP // blk
    n = ng * bps
    pix = 2 * blk * _GROUP
    rpg = _STRIP // _RD_ROWS
    nrd = ng * rpg
    lanes_pg = 2 * _GROUP // _WR_SPANS
    nw = ng * lanes_pg * bps
    banded = nw - lanes_pg * bps
    assert sum(_WR_PARTS) == blk

    hop = pow(nc, -1, bps)

    def order(q):
        return (q * hop) & (bps - 1)

    rank = {order(q): q for q in range(bps)}
    assert sorted(rank) == list(range(bps))

    def reads_needed(i):
        g, q = divmod(i, bps)
        front = max((nc * order(q) + v) % bps + 1 for v in range(nc))
        return g * rpg + front * blk // _RD_ROWS

    def unit(k):
        if isinstance(k, int):
            if k < banded:
                return divmod(k, bps)
            t, v = divmod(k - banded, _BAND)
            return (banded // bps + t % lanes_pg,
                    (t // lanes_pg * _BAND + v + nc - 1) % bps)
        t = jnp.maximum(k - banded, 0) >> _log2(_BAND)
        turn = lax.div(t, lanes_pg) * _BAND + (k & (_BAND - 1)) + nc - 1
        lane = banded // bps + lax.rem(t, lanes_pg)
        return (jnp.where(k < banded, k >> _log2(bps), lane),
                jnp.where(k < banded, k, turn) & (bps - 1))

    assert len({unit(k) for k in range(nw)}) == nw

    def chunks_needed(k):
        lane, b = unit(k)
        q = max(rank[(s * bps + b) // nc] for s in range(nc))
        return lane // lanes_pg * bps + q + 1

    npair = nrd - skew
    nb = 1 + (npair - tail - reads_needed(0)) // kp
    k0 = npair - tail - (nb - 1) * kp
    j1 = nb - 3
    tail_sem, wr_sem = nb % 3, (nb - 1) % 3
    assert k0 >= kp
    assert all(k0 + i * kp >= reads_needed(i) for i in range(j1))
    assert lead + kw * (n - j1) <= nw
    assert all(chunks_needed(k) <= j1 + max((k - lead) // kw, 0) for k in range(nw))

    def kernel(x_hbm, dw_hbm, pw_hbm, o_hbm, buf, dw_v, pw_v, sem):
        def ds(start, size, align):
            if not isinstance(start, int):
                start = pl.multiple_of(start, align)
            return pl.ds(start, size)

        def rd(q, prio, slot):
            half = _GROUP // 2
            sl = (pl.ds((q >> _log2(rpg)) * _GROUP + (1 - prio) * half, half),
                  slice(None), slice(None),
                  ds((q & (rpg - 1)) * _RD_ROWS, _RD_ROWS, _RD_ROWS))
            return pltpu.make_async_copy(x_hbm.at[sl], buf.at[sl], sem.at[slot])

        def rd_start(p, slot):
            rd(p + skew, 1, slot).start(priority=1)
            rd(p, 0, slot).start(priority=0)

        def rd_wait(first, count, slot):
            for u in range(count):
                rd(first + u + skew, 1, slot).wait()
                rd(first + u, 0, slot).wait()

        def wr(k):
            lane, b = unit(k)
            r0, cps = b * blk, []
            for size in _WR_PARTS:
                sl = (pl.ds((lane >> 1) * _WR_SPANS, _WR_SPANS), slice(None),
                      lane & 1, ds(r0, size, _SUB))
                cps.append(
                    pltpu.make_async_copy(buf.at[sl], o_hbm.at[sl], sem.at[wr_sem]))
                r0 = r0 + size
            return cps

        def wr_start(k):
            for cp in wr(k):
                cp.start()

        def wr_wait(first, count):
            for u in range(count):
                for cp in wr(first + u):
                    cp.wait()

        def each(lo, hi, fn):
            def body(i, carry):
                fn(i)
                return carry
            lax.fori_loop(lo, hi, body, 0)

        def compute(i, start_copies):
            spans = pl.ds((i >> _log2(bps)) * _GROUP, _GROUP)
            blocks = []
            for first_strip in (0, nc):
                for v in range(nc):
                    b = nc * order(i) + v
                    strip = first_strip + (b >> _log2(bps))
                    blocks.append((spans, strip >> 1, strip & 1,
                                   ds((b & (bps - 1)) * blk, blk, blk)))
            tiles = jnp.concatenate([buf[sl] for sl in blocks], axis=1)
            start_copies()
            tiles = tiles.astype(jnp.float32).reshape(pix // _SUB, nc, _SUB, _LANES)
            scale = dw_v[...].astype(jnp.float32)
            xs = jnp.concatenate(
                [(tiles[:, b].reshape(pix, _LANES)
                  * scale[:, b * _LANES:(b + 1) * _LANES]).astype(buf.dtype)
                 for b in range(nc)], axis=1)
            y = jnp.dot(xs, pw_v[...], preferred_element_type=jnp.float32)
            y = jnp.concatenate(
                [y[:, b * _LANES:(b + 1) * _LANES].reshape(pix // _SUB, 1, _SUB, _LANES)
                 for b in range(nc)], axis=1)
            y = y.reshape(_GROUP, len(blocks) * blk, _LANES).astype(buf.dtype)
            for u, sl in enumerate(blocks):
                buf[sl] = y[:, u * blk:(u + 1) * blk]

        cp_dw = pltpu.make_async_copy(dw_hbm, dw_v, sem.at[0])
        cp_pw = pltpu.make_async_copy(pw_hbm, pw_v, sem.at[0])
        cp_dw.start()
        cp_pw.start()
        each(0, skew, lambda q: rd(q, 1, 0).start(priority=1))
        each(0, k0, lambda p: rd_start(p, 0))
        each(k0, k0 + kp, lambda p: rd_start(p, 1))
        each(k0 + kp, k0 + 2 * kp, lambda p: rd_start(p, 2))
        cp_dw.wait()
        cp_pw.wait()
        for q in range(skew):
            rd(q, 1, 0).wait()
        rd_wait(0, k0 - kp, 0)

        def read_step(i, slot):
            rd_wait(k0 + (i - 1) * kp, kp, slot)

            def start_copies():
                for u in range(kp):
                    rd_start(k0 + (i + 2) * kp + u, slot)

            compute(i, start_copies)
            return jnp.where(slot == 2, 0, slot + 1)

        lax.fori_loop(0, j1, read_step, 0)

        rd_wait(k0 + (j1 - 1) * kp, kp, tail_sem)
        each(npair - tail, npair, lambda p: rd_start(p, tail_sem))
        each(npair, nrd, lambda q: rd(q, 0, tail_sem).start(priority=0))
        for b in range(j1 + 1, nb):
            rd_wait(k0 + (b - 1) * kp, kp, b % 3)
        each(0, lead, wr_start)
        rd_wait(npair - tail, tail, tail_sem)
        for q in range(npair, nrd):
            rd(q, 0, tail_sem).wait()

        def write_step(i):
            first = lead + kw * (i - j1)
            wr_wait(first - lead, kw)

            def start_copies():
                for u in range(kw):
                    wr_start(first + u)

            compute(i, start_copies)

        each(j1, n, write_step)

        def wr_next(k):
            wr_wait(k - lead, 1)
            wr_start(k)

        each(lead + kw * (n - j1), nw, wr_next)
        wr_wait(nw - lead, lead)

    xt = x.reshape(m // _SUB, _SUB, nc, _LANES).transpose(0, 2, 1, 3).reshape(view)
    out = pl.pallas_call(
        kernel,
        in_specs=[pl.BlockSpec(memory_space=pl.ANY)] * 3,
        out_specs=pl.BlockSpec(memory_space=pl.ANY),
        out_shape=jax.ShapeDtypeStruct(view, x.dtype),
        scratch_shapes=[
            pltpu.VMEM(view, x.dtype),
            pltpu.VMEM((1, c), dw.dtype),
            pltpu.VMEM((c, c), pw.dtype),
            pltpu.SemaphoreType.DMA((3,)),
        ],
        compiler_params=pltpu.CompilerParams(
            vmem_limit_bytes=124 * 1024 * 1024,
            disable_bounds_checks=True,
        ),
    )(xt, dw.reshape(1, c), pw)
    out = out.reshape(m // _SUB, nc, _SUB, _LANES).transpose(0, 2, 1, 3)
    return out.reshape(x.shape)
```
